```python
import os as _os
_os.environ.setdefault("JAX_PLATFORMS", "cpu")
import jax
import jax.numpy as jnp

def _softmax(x, axis=-1):
    return jax.nn.softmax(x, axis=axis)
def _gelu(x):
    return jax.nn.gelu(x, approximate=True)
def _silu(x):
    return jax.nn.silu(x)
def _sigmoid(x):
    return jax.nn.sigmoid(x)
def _layernorm(x, axis=-1, eps=1e-5):
    m = jnp.mean(x, axis=axis, keepdims=True)
    v = jnp.var(x, axis=axis, keepdims=True)
    return (x - m) / jnp.sqrt(v + eps)
def _scatter_add(tgt, idx, src, axis=0):
    return tgt.at[idx].add(src)
def _segment_sum(src, seg, n):
    return jax.ops.segment_sum(src, seg, n)
class _Rng:
    def __init__(self, key):
        self._k = key
    def _next(self):
        self._k, sub = jax.random.split(self._k)
        return sub
    def normal(self, shape):
        return jax.random.normal(self._next(), shape, dtype=jnp.bfloat16)
    def randint(self, lo, hi, shape):
        return jax.random.randint(self._next(), shape, lo, hi, dtype=jnp.int32)
    def uniform(self, shape, lo=0.0, hi=1.0):
        return jax.random.uniform(self._next(), shape, jnp.bfloat16, lo, hi)
    def permutation(self, n):
        return jax.random.permutation(self._next(), n)


kernel_name = 'parallel_sum__grouped_kv_mqa__dense_activation_silu__prompt'

def setup_inputs():
    _rng = _Rng(jax.random.key(int.from_bytes(__import__("os").urandom(4), "little")))
    _w = (lambda a: (lambda t: t.astype(jnp.bfloat16) if jnp.issubdtype(t.dtype, jnp.floating) else t)(jnp.asarray(a)))
    def _A_setup():
        B, S, D, H = 1, 2048, 512, 32
        Dh = D // H
        return {
            "x": _w((lambda *s: _rng.normal(s) * 0.05)(B, S, D)),
            "wq": _w((lambda *s: _rng.normal(s) * 0.05)(D, H * Dh)),
            "wk": _w((lambda *s: _rng.normal(s) * 0.05)(D, Dh)),
            "wv": _w((lambda *s: _rng.normal(s) * 0.05)(D, Dh)),
            "wo": _w((lambda *s: _rng.normal(s) * 0.05)(H * Dh, D)),
        }
    _A_in = _A_setup()

    def _B_setup():
        B, S, D, F = 1, 2048, 512, 1376
        return {
            "x": _w((lambda *s: _rng.normal(s) * 0.05)(B, S, D)),
            "w1": _w((lambda *s: _rng.normal(s) * 0.05)(D, F) * (D ** -0.5)),
            "w2": _w((lambda *s: _rng.normal(s) * 0.05)(F, D) * (F ** -0.5)),
        }
    _B_in = _B_setup()

    return {
        "A_x": _A_in["x"],
        "A_wq": _A_in["wq"],
        "A_wk": _A_in["wk"],
        "A_wv": _A_in["wv"],
        "A_wo": _A_in["wo"],
        "B_x": _B_in["x"],
        "B_w1": _B_in["w1"],
        "B_w2": _B_in["w2"],
    }

def reference(A_x, A_wq, A_wk, A_wv, A_wo, B_x, B_w1, B_w2):
    def _A_ref(x, wq, wk, wv, wo):
        B, S, D = x.shape
        H = 32
        Dh = D // H
        q = (lambda x, *d: x.transpose(*d))((x @ wq).reshape(B, S, H, Dh), 0, 2, 1, 3)
        k = x @ wk
        v = x @ wv
        scores = jnp.einsum("bhqd,bkd->bhqk", q, k) * (Dh ** -0.5)
        p = _softmax(scores, axis=-1)
        o = jnp.einsum("bhqk,bkd->bhqd", p, v)
        return (lambda x, *d: x.transpose(*d))(o, 0, 2, 1, 3).reshape(B, S, H * Dh) @ wo

    def _B_ref(x, w1, w2):
        h = jnp.einsum("bsd,df->bsf", x, w1)
        h = _silu(h)
        out = jnp.einsum("bsf,fd->bsd", h, w2)
        return out

    x = A_x
    xn = _layernorm(x, axis=-1)
    return x + _A_ref(xn, A_wq, A_wk, A_wv, A_wo) + _B_ref(xn, B_w1, B_w2)
```

```python
import functools

import jax
import jax.numpy as jnp
import jax.experimental.pallas as pl
import jax.experimental.pallas.tpu as pltpu

S = 2048
D = 512
H = 32
DH = 16
F = 1376
TB = 256
NTB = S // TB
QB = 128
NQB = S // QB
HG = 4
NC = HG * QB
UPB = H // HG
LOG2E = 1.4426950408889634
QSCALE = LOG2E * (DH ** -0.5)
MAGIC = 12582912.0
EPS = 1e-5
BOUND = 96.0
VBOUND = 2.0 ** 20

f32 = jnp.float32
i32 = jnp.int32
u32 = jnp.uint32
bf16 = jnp.bfloat16
NT = (((1,), (1,)), ((), ()))

W_SCHED = {
    2: ('f1', 0), 3: ('f1', 1), 4: ('f1', 2), 5: ('f1', 3), 6: ('o', 3), 7: ('f2', 0), 8: ('f2', 1),
    9: ('f1', 4), 10: ('f2', 2), 11: ('f1', 5), 12: ('f2', 3), 13: ('f1', 6), 14: ('o', 0),
    15: ('f2', 4), 16: ('f1', 7), 17: ('f2', 5), 18: ('f1', 8), 19: ('f2', 6), 20: ('f1', 9),
    21: ('f2', 7), 22: ('o', 1), 23: ('f1', 10), 24: ('f2', 8), 25: ('f2', 9), 28: ('f2', 10),
    30: ('o', 2),
}


def _bits(x):
    return pltpu.bitcast(x, i32)


def _exp_bits(a):
    return _bits(jnp.clip(a, 2.0 ** -60, 2.0 ** 59)) & jnp.int32(0x7F800000)


def _silu(h):
    t = 0.5 * h
    return t + t * jnp.tanh(t)


def _merge(mxu_tasks, vpu_tasks):
    done = 0
    for i, t in enumerate(mxu_tasks):
        t()
        tgt = (i + 1) * len(vpu_tasks) // len(mxu_tasks)
        while done < tgt:
            vpu_tasks[done]()
            done += 1


def _kernel(x_hbm, wq_hbm, wkt_hbm, wvt_hbm, wo_hbm, w1t_hbm, w2_hbm, o_hbm,
            x_ref, wq_ref, o_ref,
            wt_ref, ms_ref, sc_ref, xa_ref, xb_ref, xn_ref, q8_ref, mg_ref, kt_ref, vt_ref, k8_ref, kb_ref,
            acc_ref, oev_ref, on_ref, pa_ref, pb_ref, l_ref, st_ref, ks_ref, w1p_ref, w2p_ref, wop_ref,
            xsem, wsem, osem):
    def al(v, m):
        return v if isinstance(v, int) else pl.multiple_of(v, m)

    def x_copy(tb):
        r0 = al(tb * TB, TB)
        return pltpu.make_async_copy(x_hbm.at[pl.ds(r0, TB), :], x_ref.at[pl.ds(r0, TB), :], xsem.at[tb])

    wcopies = [
        pltpu.make_async_copy(wq_hbm, wq_ref, wsem.at[0]),
        pltpu.make_async_copy(wkt_hbm.bitcast(u32), wt_ref.at[D // 2:D // 2 + 8, :], wsem.at[1]),
        pltpu.make_async_copy(wvt_hbm.bitcast(u32), wt_ref.at[D // 2 + 8:D // 2 + 16, :], wsem.at[2]),
        pltpu.make_async_copy(w1t_hbm.bitcast(u32), w1p_ref, wsem.at[3]),
        pltpu.make_async_copy(w2_hbm.bitcast(u32), w2p_ref, wsem.at[4]),
        pltpu.make_async_copy(wo_hbm.bitcast(u32), wop_ref, wsem.at[5]),
    ]
    x_copy(0).start()
    for c in wcopies[:3]:
        c.start()
    for tb in range(1, NTB):
        x_copy(tb).start()
    for c in wcopies[3:]:
        c.start()

    def o_copy(b):
        r0 = al(b * QB, QB)
        return pltpu.make_async_copy(o_ref.at[pl.ds(r0, QB), :], o_hbm.at[pl.ds(r0, QB), :], osem.at[b])

    LNR = 64

    def ln_piece(tb, r, dst):
        r0 = al(tb * TB + r, LNR)
        x = x_ref[pl.ds(r0, LNR), :].astype(f32)
        mu = jnp.mean(x, axis=-1, keepdims=True)
        xc = x - mu
        var = jnp.mean(xc * xc, axis=-1, keepdims=True)
        xn = (xc * jax.lax.rsqrt(var + EPS)).astype(bf16)
        xp = pltpu.bitcast(xn, u32)
        xn_ref[pl.ds(al(r0 // 2, LNR // 2), LNR // 2), :] = xp
        dst[r // 2:(r + LNR) // 2, :] = xp

    def ln_tasks(tb, dst):
        return [functools.partial(ln_piece, tb, r, dst) for r in range(0, TB, LNR)]

    def xn_rows(r0, n):
        return pltpu.bitcast(xn_ref[pl.ds(al(r0 // 2, n // 2), n // 2), :], bf16)

    def wrows(ref, r0, n):
        return pltpu.bitcast(ref[r0 // 2:(r0 + n) // 2, :], bf16)

    rne = lambda v: (v + MAGIC) - MAGIC

    def kv_limbs(tb, kv):
        k = kv[0:DH, :]
        v = kv[DH:2 * DH, :]
        kt_ref[tb] = k
        vt_ref[tb] = pltpu.bitcast(v.astype(bf16), u32)
        ka = jnp.abs(k)
        k1 = jnp.sum(ka, axis=0, keepdims=True)
        va = jnp.max(jnp.abs(v), axis=0, keepdims=True)
        for o in range(0, TB, 128):
            st_ref[8:9, :] = jnp.maximum(st_ref[8:9, :], k1[:, o:o + 128])
            st_ref[9:10, :] = jnp.maximum(st_ref[9:10, :], va[:, o:o + 128])
        kmax = jnp.max(ka, axis=(0, 1), keepdims=True)
        ebk = _exp_bits(kmax * (1024.0 / 635.0))
        ks_ref[tb] = jnp.broadcast_to(ebk + jnp.int32(((135 - 254) << 23) + 0x400000), (8, 128))
        z = k * (pltpu.bitcast(jnp.int32(254 << 23) - ebk, f32) * 512.0)
        cc = rne(z)
        rows = []
        rem = cc
        for n in (5, 4, 3, 2):
            c = rne(rem * (1.0 / n))
            rows.append(c)
            rem = rem - c
        rows.append(rem)
        u1 = rne(cc * (1.0 / 64.0))
        u2 = rne((cc - 64.0 * u1) * 0.125)
        k8t = jnp.concatenate(rows + [rne((z - cc) * 16.0), u1, u2], axis=0)
        k8_ref[pl.ds(al(tb * TB, TB), TB), :] = _bits(k8t.T + MAGIC).astype(jnp.int8)

    kvs = []

    def q_piece(tb, j, c, s0):
        b = tb * (TB // QB) + j
        slot = s0 + j * 4 + c
        nr = 64 + (DH if c == 3 else 0)
        w = pltpu.bitcast(wt_ref[c * 64:c * 64 + nr, :], bf16)
        q = jax.lax.dot_general(w, wrows(xb_ref if s0 else xa_ref, j * QB, QB), NT, preferred_element_type=f32)
        if c == 3:
            kvs.append(q[128:160, :])
            q = q[0:128, :]
            if len(kvs) == TB // QB:
                kv_limbs(tb, jnp.concatenate(kvs, axis=1))
                kvs.clear()
        ms_ref[slot] = jnp.max(jnp.abs(q).reshape(8, 2, 8, QB), axis=1).reshape(64, QB)
        amax = ms_ref[slot, pl.ds(0, 8, stride=8), :]
        for r in range(1, 8):
            amax = jnp.maximum(amax, ms_ref[slot, pl.ds(r, 8, stride=8), :])
        st_ref[0:8, :] = jnp.maximum(st_ref[0:8, :], amax)
        eb = _exp_bits(amax * (QSCALE * 128.0 / 127.0))
        mg_ref[b, c] = eb
        sc_ref[slot] = pltpu.bitcast(jnp.int32(254 << 23) - eb, f32) * (64.0 * QSCALE)
        for h in range(8):
            t = _bits(q[h * DH:(h + 1) * DH, :] * sc_ref[slot, h:h + 1, :] + (MAGIC / 64.0 + 0.5))
            a = t >> 6
            b1 = (t & 63) - 32
            u = (t + (512 - 32)) >> 10
            b2 = (b1 + 4) >> 3
            q8_ref[b, c * 8 + h] = jnp.concatenate([a, a, a, u, b1, b2], axis=0).astype(jnp.int8)

    def q_tasks(tb, s0):
        return [functools.partial(q_piece, tb, j, c, s0) for c in (3, 0, 1, 2) for j in range(TB // QB)]

    st_ref[...] = jnp.zeros_like(st_ref)
    acc_ref[...] = jnp.zeros_like(acc_ref)
    oev_ref[...] = jnp.zeros_like(oev_ref)
    l_ref[...] = jnp.ones_like(l_ref)
    pb_ref[...] = jnp.zeros_like(pb_ref)
    x_copy(0).wait()
    for t in ln_tasks(0, xa_ref):
        t()
    for c in wcopies[:3]:
        c.wait()
    wt_ref[0:D // 2, :] = pltpu.bitcast(wq_ref[...].T, u32)

    def pre(i, c):
        tb = 2 * i
        nxt = jnp.minimum(tb + 2, NTB - 1)
        x_copy(tb + 1).wait()

        @pl.when(tb + 2 < NTB)
        def _():
            x_copy(nxt).wait()

        _merge(q_tasks(tb, 0), ln_tasks(tb + 1, xb_ref))
        _merge(q_tasks(tb + 1, 8), ln_tasks(nxt, xa_ref))
        return c

    jax.lax.fori_loop(0, NTB // 2, pre, 0)
    for c in wcopies[3:]:
        c.wait()

    def vt_tile(off, n):
        return pltpu.bitcast(vt_ref[off // TB, :, off % TB:off % TB + n], bf16)

    def finish(g, acc, l8, z=0):
        l = jnp.sum(l8, axis=0, keepdims=True)
        o = acc * (1.0 / l)
        if g % 2 == 0:
            oev_ref[...] = o
        else:
            e = oev_ref[...]
            t = jnp.concatenate([e[:, i * QB:(i + 1) * QB] for i in range(HG)]
                                + [o[:, i * QB:(i + 1) * QB] for i in range(HG)], axis=0)
            on_ref[g // 2 + z] = pltpu.bitcast(t.T.astype(bf16), u32)

    def qk_group(q8, mgq, pw, z, off, ck):
        s = jnp.dot(k8_ref[off:off + ck, :], q8, preferred_element_type=i32)
        ls = None
        for o in range(0, ck, TB):
            mg = (mgq + jnp.concatenate([ks_ref[(off + o) // TB]] * HG, axis=1))[None]
            sv = s[o:o + TB].reshape(TB // 8, 8, NC)
            p = jnp.exp2(pltpu.bitcast(sv + mg, f32) - pltpu.bitcast(mg, f32))
            pw[pl.ds(pl.multiple_of(z + (off + o) // 2, 8), TB // 2), :] = pltpu.bitcast(
                p.reshape(TB, NC).astype(bf16), u32)
            l1 = jnp.sum(p, axis=0)
            ls = l1 if ls is None else ls + l1
        return ls

    def pv_tile(pr, off):
        pp = pltpu.bitcast(pr[off // 2:off // 2 + 64, :], bf16)
        return jnp.dot(vt_tile(off, 128), pp, preferred_element_type=f32)

    def o_piece(c, bprev):
        a = jnp.dot(pltpu.bitcast(on_ref[c], bf16), wrows(wop_ref, c * 128, 128),
                    preferred_element_type=f32)
        if c == 3:
            o_ref[pl.ds(al(bprev * QB, QB), QB), :] = (acc_ref[...] + a).astype(o_ref.dtype)
        else:
            acc_ref[...] += a

    def body(b, carry):
        z = (b // 100000) * 8
        r0 = pl.multiple_of(b * QB, QB)
        bprev = jnp.maximum(b - 1, 0)
        hs = {}

        def w_piece(kind, k):
            if kind == 'o':
                o_piece(k, bprev)
            elif kind == 'f1':
                n = min(128, F - k * 128)
                h = jax.lax.dot_general(xn_rows(r0, QB), wrows(w1p_ref, k * 128, n), NT,
                                        preferred_element_type=f32)
                hs[k] = _silu(h).astype(bf16)
            else:
                n = min(128, F - k * 128)
                y = jnp.dot(hs.pop(k), wrows(w2p_ref, k * 128, n), preferred_element_type=f32)
                if k == 0:
                    acc_ref[...] = x_ref[pl.ds(r0, QB), :].astype(f32) + y
                else:
                    acc_ref[...] += y

        for j in range(UPB):
            up = (j - 1) % UPB
            pw = pa_ref if j % 2 == 0 else pb_ref
            pr = pb_ref if j % 2 == 0 else pa_ref
            v01 = jnp.concatenate([q8_ref[b, j * HG + i, 0:32, :] for i in range(HG)], axis=1)
            v23 = jnp.concatenate([q8_ref[b, j * HG + i, 32:96, :] for i in range(HG)], axis=1)
            q8 = jnp.concatenate([v01, v01, v23], axis=0)
            mgq = jnp.concatenate([jnp.broadcast_to(mg_ref[b, j // 2, (j % 2) * HG + i:(j % 2) * HG + i + 1, :], (8, QB)) for i in range(HG)], axis=1)
            l8 = None
            acc = None
            for r in range(4):
                wp = W_SCHED.get(4 * j + r)
                off = r * 512
                seq = ([('qk', off, 512), ('pv', off), ('w',), ('pv', off + 128), ('pv', off + 256), ('pv', off + 384)]
                       if wp is not None else
                       [('qk', off, 256), ('pv', off), ('pv', off + 128),
                        ('qk', off + 256, 256), ('pv', off + 256), ('pv', off + 384)])
                for op in seq:
                    if op[0] == 'qk':
                        ls = qk_group(q8, mgq, pw, z, op[1], op[2])
                        l8 = ls if l8 is None else l8 + ls
                    elif op[0] == 'pv':
                        d = pv_tile(pr, op[1])
                        acc = d if acc is None else d + acc
                    else:
                        w_piece(*wp)
            finish(up, acc, l_ref[up % 2], z)
            l_ref[j % 2] = l8

        @pl.when(b > 0)
        def _():
            o_copy(bprev).start()

        return carry

    jax.lax.fori_loop(0, NQB, body, 0)

    acc = None
    for off in range(0, S, 128):
        d = pv_tile(pb_ref, off)
        acc = d if acc is None else d + acc
    finish(UPB - 1, acc, l_ref[1])
    o_piece(3, NQB - 1)
    o_copy(NQB - 1).start()
    qm = jnp.max(st_ref[0:8, :]) * QSCALE
    km = jnp.max(st_ref[8:9, :])
    vm = jnp.max(st_ref[9:10, :])
    fast = jnp.logical_and(jnp.logical_and(qm * km <= BOUND, vm <= VBOUND),
                           jnp.logical_and(qm < 2.0 ** 50, km < 2.0 ** 50))
    for b in range(NQB):
        o_copy(b).wait()

    @pl.when(jnp.logical_not(fast))
    def _():
        CK = TB
        for tb in range(NTB):
            kbt = jnp.concatenate([kt_ref[tb], jnp.zeros((128 - DH, TB), f32)], axis=0)
            kb_ref[tb * TB:(tb + 1) * TB, :] = kbt.T.astype(bf16)

        def blk(b, c):
            r0 = pl.multiple_of(b * QB, QB)
            h = jax.lax.dot_general(xn_rows(r0, QB), wrows(w1p_ref, 0, F), NT, preferred_element_type=f32)
            y = jnp.dot(_silu(h).astype(bf16), wrows(w2p_ref, 0, F), preferred_element_type=f32)
            acc_ref[...] = x_ref[pl.ds(r0, QB), :].astype(f32) + y
            for g in range(UPB):
                w = pltpu.bitcast(wt_ref[g * 32:(g + 1) * 32, :], bf16)
                qt = jax.lax.dot_general(w, xn_rows(r0, QB), NT, preferred_element_type=f32) * QSCALE
                q = jnp.concatenate([jnp.concatenate([qt[i * DH:(i + 1) * DH] for i in range(HG)], axis=1),
                                     jnp.zeros((128 - DH, NC), f32)], axis=0).astype(bf16)

                def mx(j, m):
                    o = pl.multiple_of(j * CK, CK)
                    s = jnp.dot(kb_ref[pl.ds(o, CK), :], q, preferred_element_type=f32)
                    return jnp.maximum(m, jnp.max(s.reshape(CK // 8, 8, NC), axis=0))

                m8 = jax.lax.fori_loop(0, S // CK, mx, jnp.full((8, NC), -jnp.inf, f32))
                m = jnp.max(m8, axis=0, keepdims=True)

                def ex(j, carry):
                    acc, l8 = carry
                    o = pl.multiple_of(j * CK, CK)
                    s = jnp.dot(kb_ref[pl.ds(o, CK), :], q, preferred_element_type=f32)
                    p = jnp.exp2(s - m)
                    l8 = l8 + jnp.sum(p.reshape(CK // 8, 8, NC), axis=0)
                    vt = pltpu.bitcast(vt_ref[j], bf16)
                    acc = acc + jnp.dot(vt, p.astype(bf16), preferred_element_type=f32)
                    return acc, l8

                acc, l8 = jax.lax.fori_loop(0, S // CK, ex,
                                            (jnp.zeros((DH, NC), f32), jnp.zeros((8, NC), f32)))
                finish(g, acc, l8)
            for cc in range(4):
                o_piece(cc, b)
            cp = o_copy(b)
            cp.start()
            cp.wait()
            return c

        jax.lax.fori_loop(0, NQB, blk, 0)


@jax.jit
def pallas_parallel_sum__grouped_kv_mqa__dense_activation_silu__prompt_kernel(
        A_x, A_wq, A_wk, A_wv, A_wo, B_x, B_w1, B_w2):
    x = A_x.reshape(S, D)
    hbm = pl.BlockSpec(memory_space=pl.ANY)
    out = pl.pallas_call(
        _kernel,
        in_specs=[hbm] * 7,
        out_specs=hbm,
        out_shape=jax.ShapeDtypeStruct((S, D), A_x.dtype),
        scratch_shapes=[
            pltpu.VMEM((S, D), bf16),
            pltpu.VMEM((D, D), bf16),
            pltpu.VMEM((S, D), bf16),
            pltpu.VMEM((D // 2 + DH, D), u32),
            pltpu.VMEM((16, 64, QB), f32),
            pltpu.VMEM((16, 8, QB), f32),
            pltpu.VMEM((TB // 2, D), u32),
            pltpu.VMEM((TB // 2, D), u32),
            pltpu.VMEM((S // 2, D), u32),
            pltpu.VMEM((NQB, H, 96, QB), jnp.int8),
            pltpu.VMEM((NQB, 4, 8, QB), i32),
            pltpu.VMEM((NTB, DH, TB), f32),
            pltpu.VMEM((NTB, DH // 2, TB), u32),
            pltpu.VMEM((S, 128), jnp.int8),
            pltpu.VMEM((S, 128), bf16),
            pltpu.VMEM((QB, D), f32),
            pltpu.VMEM((DH, NC), f32),
            pltpu.VMEM((4, QB // 2, 128), u32),
            pltpu.VMEM((S // 2, NC), u32),
            pltpu.VMEM((S // 2, NC), u32),
            pltpu.VMEM((2, 8, NC), f32),
            pltpu.VMEM((16, 128), f32),
            pltpu.VMEM((NTB, 8, 128), i32),
            pltpu.VMEM((F // 2, D), u32),
            pltpu.VMEM((F // 2, D), u32),
            pltpu.VMEM((D // 2, D), u32),
            pltpu.SemaphoreType.DMA((NTB,)),
            pltpu.SemaphoreType.DMA((6,)),
            pltpu.SemaphoreType.DMA((NQB,)),
        ],
        compiler_params=pltpu.CompilerParams(vmem_limit_bytes=100 * 1024 * 1024),
    )(x, A_wq, A_wk.T, A_wv.T, A_wo, B_w1.T, B_w2)
    return out.reshape(1, S, D)
```

```python
import functools

import jax
import jax.numpy as jnp
import jax.experimental.pallas as pl
import jax.experimental.pallas.tpu as pltpu

S = 2048
D = 512
H = 32
DH = 16
F = 1376
TB = 256
NTB = S // TB
QB = 128
NQB = S // QB
HG = 4
NC = HG * QB
UPB = H // HG
LOG2E = 1.4426950408889634
QSCALE = LOG2E * (DH ** -0.5)
MAGIC = 12582912.0
EPS = 1e-5
BOUND = 96.0
NBOUND = 32.0
VBOUND = 2.0 ** 16

f32 = jnp.float32
i32 = jnp.int32
u32 = jnp.uint32
bf16 = jnp.bfloat16
NT = (((1,), (1,)), ((), ()))


def _sched():
    seq = ([('f1', 0), ('f1', 1), ('f1', 2), ('o', 3), ('f2', 0), ('f1', 3), ('f2', 1), ('f1', 4), ('f2', 2)]
           + [('f1', 5), ('o', 0), ('f2', 3), ('f1', 6), ('f2', 4), ('f1', 7), ('f2', 5), ('f1', 8)]
           + [('f2', 6), ('o', 1), ('f1', 9), ('f2', 7), ('f1', 10), ('f2', 8), ('f2', 9), ('f2', 10), ('o', 2)])
    it = iter(seq)
    out = []
    for j in range(UPB):
        if j == 0:
            out.append([(3, None)] * 4 + [(4, next(it))])
        elif j == UPB - 1:
            out.append([(3, None)] * 4 + [(4, next(it))])
        else:
            out.append([(4, next(it)) for _ in range(4)])
    return out


SCHED = _sched()


def _bits(x):
    return pltpu.bitcast(x, i32)


def _exp_bits(a):
    return _bits(jnp.clip(a, 2.0 ** -60, 2.0 ** 59)) & jnp.int32(0x7F800000)


def _silu(h):
    t = 0.5 * h
    return t + t * jnp.tanh(t)


def _kernel(x_hbm, wq_hbm, wkt_hbm, wvt_hbm, wo_hbm, w1t_hbm, w2_hbm, o_hbm,
            x_ref, wq_ref, o_ref,
            w1t_ref, w2_ref, wo_ref, wt_ref, wkv_ref, qs_ref, ms_ref, sc_ref, xa_ref, xb_ref, xn_ref, q8_ref, mg_ref, kt_ref, vt_ref, k8_ref, kb_ref,
            acc_ref, oev_ref, on_ref, pa_ref, pb_ref, l_ref, st_ref, ks_ref, w1p_ref, w2p_ref, wop_ref,
            isem, osem):
    def al(v, m):
        return v if isinstance(v, int) else pl.multiple_of(v, m)

    def x_copy(tb):
        r0 = al(tb * TB, TB)
        return pltpu.make_async_copy(x_hbm.at[pl.ds(r0, TB), :], x_ref.at[pl.ds(r0, TB), :], isem.at[6 + tb])

    wcopies = [
        pltpu.make_async_copy(wq_hbm, wq_ref, isem.at[0]),
        pltpu.make_async_copy(wkt_hbm, wkv_ref.at[0:DH, :], isem.at[1]),
        pltpu.make_async_copy(wvt_hbm, wkv_ref.at[DH:2 * DH, :], isem.at[2]),
        pltpu.make_async_copy(w1t_hbm, w1t_ref, isem.at[3]),
        pltpu.make_async_copy(w2_hbm, w2_ref, isem.at[4]),
        pltpu.make_async_copy(wo_hbm, wo_ref, isem.at[5]),
    ]
    x_copy(0).start()
    for c in wcopies[:3]:
        c.start()
    for tb in range(1, NTB):
        x_copy(tb).start()
    for c in wcopies[3:]:
        c.start()

    def o_copy(b):
        r0 = al(b * QB, QB)
        return pltpu.make_async_copy(o_ref.at[pl.ds(r0, QB), :], o_hbm.at[pl.ds(r0, QB), :], osem.at[b])

    LNR = 64

    def ln_piece(tb, r, dst):
        r0 = al(tb * TB + r, LNR)
        x = x_ref[pl.ds(r0, LNR), :].astype(f32)
        mu = jnp.mean(x, axis=-1, keepdims=True)
        xc = x - mu
        var = jnp.mean(xc * xc, axis=-1, keepdims=True)
        xn = (xc * jax.lax.rsqrt(var + EPS)).astype(bf16)
        xp = pltpu.bitcast(xn, u32)
        xn_ref[pl.ds(al(r0 // 2, LNR // 2), LNR // 2), :] = xp
        dst[r // 2:(r + LNR) // 2, :] = xp

    def ln_tasks(tb, dst):
        return [functools.partial(ln_piece, tb, r, dst) for r in range(0, TB, LNR)]

    def xn_rows(r0, n):
        return pltpu.bitcast(xn_ref[pl.ds(al(r0 // 2, n // 2), n // 2), :], bf16)

    def wrows(ref, r0, n):
        return pltpu.bitcast(ref[r0 // 2:(r0 + n) // 2, :], bf16)

    rne = jnp.round

    def kv_limbs(tb, kv):
        k = kv[0:DH, :]
        v = kv[DH:2 * DH, :]
        kt_ref[tb] = k
        vt_ref[tb] = pltpu.bitcast(v.astype(bf16), u32)
        ka = jnp.abs(k)
        k1 = jnp.sum(ka, axis=0, keepdims=True)
        va = jnp.max(jnp.abs(v), axis=0, keepdims=True)
        for o in range(0, TB, 128):
            st_ref[8:9, :] = jnp.maximum(st_ref[8:9, :], k1[:, o:o + 128])
            st_ref[9:10, :] = jnp.maximum(st_ref[9:10, :], va[:, o:o + 128])
        kmax = jnp.max(ka, axis=(0, 1), keepdims=True)
        st_ref[10:11, :] = jnp.maximum(st_ref[10:11, :], jnp.broadcast_to(kmax, (1, 128)))
        ebk = _exp_bits(kmax * (1024.0 / 635.0))
        ks_ref[tb] = jnp.broadcast_to(ebk + jnp.int32(((135 - 254) << 23) + 0x400000), (8, 128))
        z = k * (pltpu.bitcast(jnp.int32(254 << 23) - ebk, f32) * 512.0)
        cc = rne(z)
        rows = []
        rem = cc
        for n in (5, 4, 3, 2):
            c = rne(rem * (1.0 / n))
            rows.append(c)
            rem = rem - c
        rows.append(rem)
        u1 = rne(cc * (1.0 / 64.0))
        u2 = rne((cc - 64.0 * u1) * 0.125)
        k8t = jnp.concatenate(rows + [rne((z - cc) * 16.0), u1, u2], axis=0)
        k8_ref[pl.ds(al(tb * TB, TB), TB), :] = _bits(k8t.T + MAGIC).astype(jnp.int8)

    kvs = []

    def q_stats(tb, j, c, s0):
        b = tb * (TB // QB) + j
        slot = s0 + j * 4 + c
        amax = ms_ref[slot, pl.ds(0, 8, stride=8), :]
        for r in range(1, 8):
            amax = jnp.maximum(amax, ms_ref[slot, pl.ds(r, 8, stride=8), :])
        st_ref[0:8, :] = jnp.maximum(st_ref[0:8, :], amax)
        eb = _exp_bits(amax * (QSCALE * 128.0 / 127.0))
        mg_ref[b, c] = eb
        sc_ref[slot] = pltpu.bitcast(jnp.int32(254 << 23) - eb, f32) * (64.0 * QSCALE)

    def q_limbs(tb, j, c, s0, h):
        b = tb * (TB // QB) + j
        slot = s0 + j * 4 + c
        t = _bits(qs_ref[slot, h * DH:(h + 1) * DH, :] * sc_ref[slot, h:h + 1, :] + (MAGIC / 64.0 + 0.5))
        a = t >> 6
        b1 = (t & 63) - 32
        u = (t + (512 - 32)) >> 10
        b2 = (b1 + 4) >> 3
        q8_ref[b, c * 8 + h] = jnp.concatenate([a, a, a, u, b1, b2], axis=0).astype(jnp.int8)

    def q_piece(cur, prev, z):
        tb, j, c, s0 = cur
        slot = s0 + j * 4 + c
        nr = 64 + (DH if c == 3 else 0)
        w = pltpu.bitcast(wt_ref[c * 64:c * 64 + nr, :], bf16)
        q = jax.lax.dot_general(w, wrows(xb_ref if s0 else xa_ref, j * QB, QB), NT, preferred_element_type=f32)
        for h in range(8):
            qh = q[h * DH:(h + 1) * DH, :]
            qs_ref[slot + z, h * DH:(h + 1) * DH, :] = qh
            ms_ref[slot, h * 8:(h + 1) * 8, :] = jnp.maximum(jnp.abs(qh[0:8]), jnp.abs(qh[8:16]))
            if prev is not None:
                q_limbs(*prev, h)
        q_stats(*cur)
        if c == 3:
            kvs.append(q[128:160, :])
            if len(kvs) == TB // QB:
                kv_limbs(tb, jnp.concatenate(kvs, axis=1))
                kvs.clear()

    st_ref[...] = jnp.zeros_like(st_ref)
    acc_ref[...] = jnp.zeros_like(acc_ref)
    oev_ref[...] = jnp.zeros_like(oev_ref)
    l_ref[...] = jnp.ones_like(l_ref)
    pb_ref[...] = jnp.zeros_like(pb_ref)
    x_copy(0).wait()
    for t in ln_tasks(0, xa_ref):
        t()
    for c in wcopies[:3]:
        c.wait()
    wt_ref[D // 2:D // 2 + DH, :] = pltpu.bitcast(wkv_ref[...], u32)
    wt_ref[0:D // 2, :] = pltpu.bitcast(wq_ref[...].T, u32)

    def pre(i, c):
        tb = 2 * i
        nxt = jnp.minimum(tb + 2, NTB - 1)
        x_copy(tb + 1).wait()

        @pl.when(tb + 2 < NTB)
        def _():
            x_copy(nxt).wait()

        z = i // 100000
        pieces = [(t, j, c, s0) for (t, s0) in ((tb, 0), (tb + 1, 8)) for c in (3, 0, 1, 2) for j in range(TB // QB)]
        lns = ln_tasks(tb + 1, xb_ref) + ln_tasks(nxt, xa_ref)
        for n, p in enumerate(pieces):
            q_piece(p, pieces[n - 1] if n else None, z)
            if n % 2 == 1:
                lns[n // 2]()
        for h in range(8):
            q_limbs(*pieces[-1], h)
        return c

    jax.lax.fori_loop(0, NTB // 2, pre, 0)
    for c, src, dst, rows in zip(wcopies[3:], (w1t_ref, w2_ref, wo_ref), (w1p_ref, w2p_ref, wop_ref), (F, F, D)):
        c.wait()

        def repack(r, carry, src=src, dst=dst):
            dst[pl.ds(pl.multiple_of(r * 16, 16), 16), :] = pltpu.bitcast(
                src[pl.ds(pl.multiple_of(r * 32, 32), 32), :], u32)
            return carry

        jax.lax.fori_loop(0, rows // 32, repack, 0, unroll=True)

    def vt_tile(off, n):
        return pltpu.bitcast(vt_ref[off // TB, :, off % TB:off % TB + n], bf16)

    def recip(l8):
        l = jnp.sum(l8, axis=0, keepdims=True)
        return jnp.broadcast_to(1.0 / l, (8, NC))

    def finish(g, acc, r8, z=0):
        o = acc * jnp.concatenate([r8, r8], axis=0)
        if g % 2 == 0:
            oev_ref[...] = o
        else:
            e = oev_ref[...]
            t = jnp.concatenate([e[:, i * QB:(i + 1) * QB] for i in range(HG)]
                                + [o[:, i * QB:(i + 1) * QB] for i in range(HG)], axis=0)
            on_ref[g // 2 + z] = pltpu.bitcast(t.T.astype(bf16), u32)

    def qk_group(q8, mgq, pw, z, off, ck):
        s = jnp.dot(k8_ref[off:off + ck, :], q8, preferred_element_type=i32)
        ls = None
        o = 0
        while o < ck:
            n = min(ck - o, TB - (off + o) % TB)
            mg = (mgq + jnp.concatenate([ks_ref[(off + o) // TB]] * HG, axis=1))[None]
            sv = s[o:o + n].reshape(n // 8, 8, NC)
            p = jnp.exp2(pltpu.bitcast(sv + mg, f32) - pltpu.bitcast(mg, f32))
            pw[pl.ds(pl.multiple_of(z + (off + o) // 2, 8), n // 2), :] = pltpu.bitcast(
                p.reshape(n, NC).astype(bf16), u32)
            l1 = jnp.sum(p, axis=0)
            ls = l1 if ls is None else ls + l1
            o += n
        return ls

    def pv_tile(pr, off):
        pp = pltpu.bitcast(pr[off // 2:off // 2 + 64, :], bf16)
        return jnp.dot(vt_tile(off, 128), pp, preferred_element_type=f32)

    def o_piece(c, bprev):
        a = jnp.dot(pltpu.bitcast(on_ref[c], bf16), wrows(wop_ref, c * 128, 128),
                    preferred_element_type=f32)
        if c == 3:
            o_ref[pl.ds(al(bprev * QB, QB), QB), :] = (acc_ref[...] + a).astype(o_ref.dtype)
        else:
            acc_ref[...] += a

    def body(b, carry):
        z = (b // 100000) * 8
        r0 = pl.multiple_of(b * QB, QB)
        bprev = jnp.maximum(b - 1, 0)
        hs = {}

        def w_piece(kind, k):
            if kind == 'o':
                o_piece(k, bprev)
            elif kind == 'f1':
                n = min(128, F - k * 128)
                h = jax.lax.dot_general(xn_rows(r0, QB), wrows(w1p_ref, k * 128, n), NT,
                                        preferred_element_type=f32)
                hs[k] = _silu(h).astype(bf16)
            else:
                n = min(128, F - k * 128)
                y = jnp.dot(hs.pop(k), wrows(w2p_ref, k * 128, n), preferred_element_type=f32)
                if k == 0:
                    acc_ref[...] = x_ref[pl.ds(r0, QB), :].astype(f32) + y
                else:
                    acc_ref[...] += y

        r8 = recip(l_ref[...])
        for j in range(UPB):
            up = (j - 1) % UPB
            pw = pa_ref if j % 2 == 0 else pb_ref
            pr = pb_ref if j % 2 == 0 else pa_ref
            v01 = jnp.concatenate([q8_ref[b, j * HG + i, 0:32, :] for i in range(HG)], axis=1)
            v23 = jnp.concatenate([q8_ref[b, j * HG + i, 32:96, :] for i in range(HG)], axis=1)
            q8 = jnp.concatenate([v01, v01, v23], axis=0)
            mgq = jnp.concatenate([jnp.broadcast_to(mg_ref[b, j // 2, (j % 2) * HG + i:(j % 2) * HG + i + 1, :], (8, QB)) for i in range(HG)], axis=1)
            l8 = None
            acc = None
            off = 0
            for nt, wp in SCHED[j]:
                seq = [('qk', off, nt * 128)] + [('pv', off + t * 128) for t in range(nt)]
                if wp is not None:
                    seq.insert(2, ('w',))
                off += nt * 128
                for op in seq:
                    if op[0] == 'qk':
                        ls = qk_group(q8, mgq, pw, z, op[1], op[2])
                        l8 = ls if l8 is None else l8 + ls
                    elif op[0] == 'pv':
                        d = pv_tile(pr, op[1])
                        acc = d if acc is None else d + acc
                    else:
                        w_piece(*wp)
            finish(up, acc, r8, z)
            if j + 1 < UPB:
                r8 = recip(l8)
            else:
                l_ref[...] = l8

        @pl.when(b > 0)
        def _():
            o_copy(bprev).start()

        return carry

    jax.lax.fori_loop(0, NQB, body, 0)

    acc = None
    for off in range(0, S, 128):
        d = pv_tile(pb_ref, off)
        acc = d if acc is None else d + acc
    finish(UPB - 1, acc, recip(l_ref[...]))
    o_piece(3, NQB - 1)
    o_copy(NQB - 1).start()
    qm = jnp.max(st_ref[0:8, :]) * QSCALE
    km = jnp.max(st_ref[8:9, :])
    vm = jnp.max(st_ref[9:10, :])
    ka = jnp.max(st_ref[10:11, :])
    fast = jnp.logical_and(jnp.logical_and(qm * km <= BOUND, vm <= VBOUND),
                           jnp.logical_and(qm < 2.0 ** 50, km < 2.0 ** 50))
    fast = jnp.logical_and(fast, qm * ka <= NBOUND)
    for b in range(NQB):
        o_copy(b).wait()

    @pl.when(jnp.logical_not(fast))
    def _():
        CK = TB
        for tb in range(NTB):
            kbt = jnp.concatenate([kt_ref[tb], jnp.zeros((128 - DH, TB), f32)], axis=0)
            kb_ref[tb * TB:(tb + 1) * TB, :] = kbt.T.astype(bf16)

        def blk(b, c):
            r0 = pl.multiple_of(b * QB, QB)
            h = jax.lax.dot_general(xn_rows(r0, QB), wrows(w1p_ref, 0, F), NT, preferred_element_type=f32)
            y = jnp.dot(_silu(h).astype(bf16), wrows(w2p_ref, 0, F), preferred_element_type=f32)
            acc_ref[...] = x_ref[pl.ds(r0, QB), :].astype(f32) + y
            for g in range(UPB):
                w = pltpu.bitcast(wt_ref[g * 32:(g + 1) * 32, :], bf16)
                qt = jax.lax.dot_general(w, xn_rows(r0, QB), NT, preferred_element_type=f32) * QSCALE
                q = jnp.concatenate([jnp.concatenate([qt[i * DH:(i + 1) * DH] for i in range(HG)], axis=1),
                                     jnp.zeros((128 - DH, NC), f32)], axis=0).astype(bf16)

                def mx(j, m):
                    o = pl.multiple_of(j * CK, CK)
                    s = jnp.dot(kb_ref[pl.ds(o, CK), :], q, preferred_element_type=f32)
                    return jnp.maximum(m, jnp.max(s.reshape(CK // 8, 8, NC), axis=0))

                m8 = jax.lax.fori_loop(0, S // CK, mx, jnp.full((8, NC), -jnp.inf, f32))
                m = jnp.max(m8, axis=0, keepdims=True)

                def ex(j, carry):
                    acc, l8 = carry
                    o = pl.multiple_of(j * CK, CK)
                    s = jnp.dot(kb_ref[pl.ds(o, CK), :], q, preferred_element_type=f32)
                    p = jnp.exp2(s - m)
                    l8 = l8 + jnp.sum(p.reshape(CK // 8, 8, NC), axis=0)
                    vt = pltpu.bitcast(vt_ref[j], bf16)
                    acc = acc + jnp.dot(vt, p.astype(bf16), preferred_element_type=f32)
                    return acc, l8

                acc, l8 = jax.lax.fori_loop(0, S // CK, ex,
                                            (jnp.zeros((DH, NC), f32), jnp.zeros((8, NC), f32)))
                finish(g, acc, recip(l8))
            for cc in range(4):
                o_piece(cc, b)
            cp = o_copy(b)
            cp.start()
            cp.wait()
            return c

        jax.lax.fori_loop(0, NQB, blk, 0)


@jax.jit
def pallas_parallel_sum__grouped_kv_mqa__dense_activation_silu__prompt_kernel(
        A_x, A_wq, A_wk, A_wv, A_wo, B_x, B_w1, B_w2):
    x = A_x.reshape(S, D)
    hbm = pl.BlockSpec(memory_space=pl.ANY)
    out = pl.pallas_call(
        _kernel,
        in_specs=[hbm] * 7,
        out_specs=hbm,
        out_shape=jax.ShapeDtypeStruct((S, D), A_x.dtype),
        scratch_shapes=[
            pltpu.VMEM((S, D), bf16),
            pltpu.VMEM((D, D), bf16),
            pltpu.VMEM((S, D), bf16),
            pltpu.VMEM((F, D), bf16),
            pltpu.VMEM((F, D), bf16),
            pltpu.VMEM((D, D), bf16),
            pltpu.VMEM((D // 2 + DH, D), u32),
            pltpu.VMEM((2 * DH, D), bf16),
            pltpu.VMEM((16, 128, QB), f32),
            pltpu.VMEM((16, 64, QB), f32),
            pltpu.VMEM((16, 8, QB), f32),
            pltpu.VMEM((TB // 2, D), u32),
            pltpu.VMEM((TB // 2, D), u32),
            pltpu.VMEM((S // 2, D), u32),
            pltpu.VMEM((NQB, H, 96, QB), jnp.int8),
            pltpu.VMEM((NQB, 4, 8, QB), i32),
            pltpu.VMEM((NTB, DH, TB), f32),
            pltpu.VMEM((NTB, DH // 2, TB), u32),
            pltpu.VMEM((S, 128), jnp.int8),
            pltpu.VMEM((S, 128), bf16),
            pltpu.VMEM((QB, D), f32),
            pltpu.VMEM((DH, NC), f32),
            pltpu.VMEM((4, QB // 2, 128), u32),
            pltpu.VMEM((S // 2, NC), u32),
            pltpu.VMEM((S // 2, NC), u32),
            pltpu.VMEM((8, NC), f32),
            pltpu.VMEM((16, 128), f32),
            pltpu.VMEM((NTB, 8, 128), i32),
            pltpu.VMEM((F // 2, D), u32),
            pltpu.VMEM((F // 2, D), u32),
            pltpu.VMEM((D // 2, D), u32),
            pltpu.SemaphoreType.DMA((6 + NTB,)),
            pltpu.SemaphoreType.DMA((NQB,)),
        ],
        compiler_params=pltpu.CompilerParams(vmem_limit_bytes=100 * 1024 * 1024),
    )(x, A_wq, A_wk.T, A_wv.T, A_wo, B_w1.T, B_w2)
    return out.reshape(1, S, D)
```
